```python
import jax
import jax.numpy as jnp

def _softmax(x, axis=-1):
    return jax.nn.softmax(x, axis=axis)
def _gelu(x):
    return jax.nn.gelu(x, approximate=True)
def _silu(x):
    return jax.nn.silu(x)
def _sigmoid(x):
    return jax.nn.sigmoid(x)
def _layernorm(x, axis=-1, eps=1e-5):
    m = jnp.mean(x, axis=axis, keepdims=True)
    v = jnp.var(x, axis=axis, keepdims=True)
    return (x - m) / jnp.sqrt(v + eps)
def _scatter_add(tgt, idx, src, axis=0):
    return tgt.at[idx].add(src)
def _segment_sum(src, seg, n):
    return jax.ops.segment_sum(src, seg, n)
class _Rng:
    def __init__(self, key):
        self._k = key
    def _next(self):
        self._k, sub = jax.random.split(self._k)
        return sub
    def normal(self, shape):
        return jax.random.normal(self._next(), shape, dtype=jnp.bfloat16)
    def randint(self, lo, hi, shape):
        return jax.random.randint(self._next(), shape, lo, hi, dtype=jnp.int32)
    def uniform(self, shape, lo=0.0, hi=1.0):
        return jax.random.uniform(self._next(), shape, jnp.bfloat16, lo, hi)
    def permutation(self, n):
        return jax.random.permutation(self._next(), n)


kernel_name = 'concat_heads__compressed_kv_cla__mha_block_cached__decode'

def setup_inputs():
    _rng = _Rng(jax.random.key(int.from_bytes(__import__("os").urandom(4), "little")))
    _w = (lambda a: (lambda t: t.astype(jnp.bfloat16) if jnp.issubdtype(t.dtype, jnp.floating) else t)(jnp.asarray(a)))
    def _A_setup():
        B, H, Sq, Sk, D, M = 4, 32, 1, 4096, 128, 512
        Dc = 4 * D
        return {
            "x": _w((lambda *s: _rng.normal(s) * 0.05)(B, Sq, M)),
            "c_kv": _w((lambda *s: _rng.normal(s) * 0.05)(B, Sk, Dc)),
            "w_q": _w((lambda *s: _rng.normal(s) * 0.05)(M, H, D) * (M ** -0.5)),
            "w_uk": _w((lambda *s: _rng.normal(s) * 0.05)(Dc, H, D) * (Dc ** -0.5)),
            "w_uv": _w((lambda *s: _rng.normal(s) * 0.05)(Dc, H, D) * (Dc ** -0.5)),
            "w_o": _w((lambda *s: _rng.normal(s) * 0.05)(H, D, M) * ((H * D) ** -0.5)),
        }
    _A_in = _A_setup()

    def _B_setup():
        B, Sq, D = 4, 1, 512
        H, Sk, Dh = 32, 4096, 128
        return {
            "x": _w((lambda *s: _rng.normal(s) * 0.05)(B, Sq, D)),
            "k_cache": _w((lambda *s: _rng.normal(s) * 0.05)(B, H, Sk, Dh)),
            "v_cache": _w((lambda *s: _rng.normal(s) * 0.05)(B, H, Sk, Dh)),
            "wq": _w((lambda *s: _rng.normal(s) * 0.05)(D, H * Dh) * (D ** -0.5)),
            "wo": _w((lambda *s: _rng.normal(s) * 0.05)(H * Dh, D) * ((H * Dh) ** -0.5)),
        }
    _B_in = _B_setup()

    return {
        "A_x": _A_in["x"],
        "A_c_kv": _A_in["c_kv"],
        "A_w_q": _A_in["w_q"],
        "A_w_uk": _A_in["w_uk"],
        "A_w_uv": _A_in["w_uv"],
        "A_w_o": _A_in["w_o"],
        "B_x": _B_in["x"],
        "B_k_cache": _B_in["k_cache"],
        "B_v_cache": _B_in["v_cache"],
        "B_wq": _B_in["wq"],
        "B_wo": _B_in["wo"],
    }

def reference(A_x, A_c_kv, A_w_q, A_w_uk, A_w_uv, A_w_o, B_x, B_k_cache, B_v_cache, B_wq, B_wo):
    def _A_ref(x, c_kv, w_q, w_uk, w_uv, w_o):
        B, Sq, M = x.shape[0], x.shape[1], x.shape[2]
        Sk = c_kv.shape[1]
        H, D = w_q.shape[1], w_q.shape[2]
        q = jnp.einsum("bqm,mhd->bhqd", x, w_q)
        k = jnp.einsum("bkc,chd->bhkd", c_kv, w_uk)
        v = jnp.einsum("bkc,chd->bhkd", c_kv, w_uv)
        scores = jnp.einsum("bhqd,bhkd->bhqk", q, k) * (D ** -0.5)
        off = Sk - Sq
        qi = jnp.arange(Sq)[:, None]
        kj = jnp.arange(Sk)[None, :]
        cmask = kj <= (qi + off)
        scores = jnp.where(cmask[None, None], scores, -1e9)
        p = _softmax(scores, axis=-1)
        ctx = jnp.einsum("bhqk,bhkd->bhqd", p, v)
        return jnp.einsum("bhqd,hdm->bqm", ctx, w_o)

    def _B_ref(x, k_cache, v_cache, wq, wo):
        B, Sq, D = x.shape
        H, Dh = 32, 128
        q = (lambda x, *d: x.transpose(*d))((x @ wq).reshape(B, Sq, H, Dh), 0, 2, 1, 3)
        scores = jnp.einsum("bhqd,bhkd->bhqk", q, k_cache) * (Dh ** -0.5)
        p = _softmax(scores, axis=-1)
        o = jnp.einsum("bhqk,bhkd->bhqd", p, v_cache)
        return (lambda x, *d: x.transpose(*d))(o, 0, 2, 1, 3).reshape(B, Sq, H * Dh) @ wo

    a = _A_ref(A_x, A_c_kv, A_w_q, A_w_uk, A_w_uv, A_w_o)
    b = _B_ref(B_x, B_k_cache, B_v_cache, B_wq, B_wo)
    return jnp.concatenate([a, b], axis=-1)
```

```python
import jax
import jax.numpy as jnp
import jax.experimental.pallas as pl
import jax.experimental.pallas.tpu as pltpu

_ROWS = 8
_LANES = 128

_NT = (((1,), (1,)), ((), ()))


def _dot(a, b):
    return jnp.dot(a, b, preferred_element_type=jnp.float32)


def _dot_nt(a, b):
    return jax.lax.dot_general(a, b, _NT, preferred_element_type=jnp.float32)


def _stack_rows(x_ref):
    nb, _, m = x_ref.shape
    row = jax.lax.broadcasted_iota(jnp.int32, (_ROWS, m), 0)
    out = jnp.zeros((_ROWS, m), jnp.float32)
    for b in range(nb):
        out = jnp.where(row == b, x_ref[b].astype(jnp.float32), out)
    return out.astype(jnp.bfloat16)


def _head_pair(w_buf, j, n, npair):
    words = w_buf[pl.ds(j, n, stride=npair), :]
    even = pltpu.bitcast(words << 16, jnp.float32)
    odd = pltpu.bitcast(words & jnp.uint32(0xFFFF0000), jnp.float32)
    return even.astype(jnp.bfloat16), odd.astype(jnp.bfloat16)


def _softmax_parts(s):
    m = jnp.max(s, axis=-1, keepdims=True)
    p = jnp.exp(s - m)
    return p.astype(jnp.bfloat16), jnp.sum(p, axis=-1, keepdims=True)


def _kernel(ax_ref, ckv_hbm, wq_hbm, wuk_hbm, wuv_hbm, wo_hbm,
            bx_ref, k_hbm, v_hbm, bwq_hbm, bwo_hbm,
            o_ref,
            wq_buf, wuk_buf, wuv_buf, wo_buf, bwq_buf, bwo_buf, ckv_buf,
            k_buf, v_buf, lat_buf, qb_buf,
            w_sem, c_sem, k_sem, v_sem):
    nb, sk, dc = ckv_hbm.shape
    nh, dh = k_hbm.shape[1], k_hbm.shape[3]
    m = ax_ref.shape[2]
    npair = nh // 2
    scale = dh ** -0.5

    wq_cp = pltpu.make_async_copy(wq_hbm.bitcast(jnp.uint32), wq_buf, w_sem.at[0])
    wuk_cp = pltpu.make_async_copy(wuk_hbm.bitcast(jnp.uint32), wuk_buf, w_sem.at[1])
    wuv_cp = pltpu.make_async_copy(wuv_hbm.bitcast(jnp.uint32), wuv_buf, w_sem.at[2])
    wo_cp = pltpu.make_async_copy(wo_hbm, wo_buf, w_sem.at[3])
    bwq_cp = pltpu.make_async_copy(bwq_hbm, bwq_buf, w_sem.at[4])
    bwo_cp = pltpu.make_async_copy(bwo_hbm, bwo_buf, w_sem.at[5])
    c_cp = [pltpu.make_async_copy(ckv_hbm.at[b], ckv_buf.at[b], c_sem.at[b])
            for b in range(nb)]

    def k_cp(b, h):
        return pltpu.make_async_copy(k_hbm.at[b, h], k_buf.at[b], k_sem.at[b])

    def v_cp(b, h):
        return pltpu.make_async_copy(v_hbm.at[b, h], v_buf.at[b], v_sem.at[b])

    def lat_store(rows, val):
        for i in range(dc // _LANES):
            lat_buf[i, rows, :] = val[:, i * _LANES:(i + 1) * _LANES]

    def lat_load(rows):
        parts = [lat_buf[i, rows, :] for i in range(dc // _LANES)]
        return jnp.concatenate(parts, axis=1).astype(jnp.bfloat16)

    wq_cp.start()
    wuk_cp.start()
    c_cp[0].start()
    xa = _stack_rows(ax_ref)
    wq_cp.wait()
    wuk_cp.wait()
    c_cp[1].start()

    def absorb(j, carry):
        wq2 = _head_pair(wq_buf, j, m, npair)
        wuk2 = _head_pair(wuk_buf, j, dc, npair)
        for t in range(2):
            q = _dot(xa, wq2[t]).astype(jnp.bfloat16)
            r0 = pl.multiple_of((2 * j + t) * _ROWS, _ROWS)
            lat_store(pl.ds(r0, _ROWS), _dot_nt(q, wuk2[t]))
        return carry

    jax.lax.fori_loop(0, npair, absorb, 0)

    nxt = [c_cp[2], c_cp[3], wuv_cp, wo_cp]
    for b in range(nb):
        nxt[b].start()
        c_cp[b].wait()
        rows = pl.ds(b, nh, stride=_ROWS)
        q_lat = lat_load(rows)
        c = ckv_buf[b]
        p, l = _softmax_parts(_dot_nt(q_lat, c) * scale)
        lat_store(rows, _dot(p, c) / l)

    bwq_cp.start()
    wuv_cp.wait()
    bwo_cp.start()
    wo_cp.wait()
    for b in range(nb):
        k_cp(b, 0).start()
        v_cp(b, 0).start()

    def project(j, acc):
        wuv2 = _head_pair(wuv_buf, j, dc, npair)
        for t in range(2):
            h = 2 * j + t
            r0 = pl.multiple_of(h * _ROWS, _ROWS)
            lat = lat_load(pl.ds(r0, _ROWS))
            ctx = _dot(lat, wuv2[t]).astype(jnp.bfloat16)
            acc = acc + _dot(ctx, wo_buf[h])
        return acc

    out_a = jax.lax.fori_loop(0, npair, project,
                              jnp.zeros((_ROWS, m), jnp.float32))

    xb = _stack_rows(bx_ref)
    bwq_cp.wait()
    for h in range(nh):
        qb_buf[h] = _dot(xb, bwq_buf[:, h * dh:(h + 1) * dh])
    bwo_cp.wait()

    row = jax.lax.broadcasted_iota(jnp.int32, (_ROWS, dh), 0)

    def head(h, acc):
        q = qb_buf[h].astype(jnp.bfloat16)
        o = jnp.zeros((_ROWS, dh), jnp.float32)
        for b in range(nb):
            k_cp(b, h).wait()
            p, l = _softmax_parts(_dot_nt(q, k_buf[b]) * scale)

            @pl.when(h + 1 < nh)
            def _():
                k_cp(b, h + 1).start()

            v_cp(b, h).wait()
            o = jnp.where(row == b, _dot(p, v_buf[b]) / l, o)

            @pl.when(h + 1 < nh)
            def _():
                v_cp(b, h + 1).start()

        r0 = pl.multiple_of(h * dh, dh)
        return acc + _dot(o.astype(jnp.bfloat16), bwo_buf[pl.ds(r0, dh), :])

    out_b = jax.lax.fori_loop(0, nh, head, jnp.zeros((_ROWS, m), jnp.float32))

    for b in range(nb):
        o_ref[b, :, 0:m] = out_a[b:b + 1, :].astype(o_ref.dtype)
        o_ref[b, :, m:2 * m] = out_b[b:b + 1, :].astype(o_ref.dtype)


@jax.jit
def pallas_concat_heads__compressed_kv_cla__mha_block_cached__decode_kernel(
    A_x: jax.Array,
    A_c_kv: jax.Array,
    A_w_q: jax.Array,
    A_w_uk: jax.Array,
    A_w_uv: jax.Array,
    A_w_o: jax.Array,
    B_x: jax.Array,
    B_k_cache: jax.Array,
    B_v_cache: jax.Array,
    B_wq: jax.Array,
    B_wo: jax.Array,
):
    nb, sq, m = A_x.shape
    _, sk, dc = A_c_kv.shape
    _, nh, dh = A_w_q.shape
    assert sq == 1 and nb <= _ROWS and nh % 2 == 0
    assert B_k_cache.shape == (nb, nh, sk, dh) and B_x.shape == A_x.shape
    bf16 = jnp.bfloat16

    hbm = pl.BlockSpec(memory_space=pl.ANY)
    vmem = pl.BlockSpec(memory_space=pltpu.VMEM)
    return pl.pallas_call(
        _kernel,
        out_shape=jax.ShapeDtypeStruct((nb, sq, 2 * m), A_x.dtype),
        in_specs=[vmem, hbm, hbm, hbm, hbm, hbm, vmem, hbm, hbm, hbm, hbm],
        out_specs=vmem,
        scratch_shapes=[
            pltpu.VMEM((m * nh // 2, dh), jnp.uint32),
            pltpu.VMEM((dc * nh // 2, dh), jnp.uint32),
            pltpu.VMEM((dc * nh // 2, dh), jnp.uint32),
            pltpu.VMEM((nh, dh, m), bf16),
            pltpu.VMEM((m, nh * dh), bf16),
            pltpu.VMEM((nh * dh, m), bf16),
            pltpu.VMEM((nb, sk, dc), bf16),
            pltpu.VMEM((nb, sk, dh), bf16),
            pltpu.VMEM((nb, sk, dh), bf16),
            pltpu.VMEM((dc // _LANES, nh * _ROWS, _LANES), jnp.float32),
            pltpu.VMEM((nh, _ROWS, dh), jnp.float32),
            pltpu.SemaphoreType.DMA((6,)),
            pltpu.SemaphoreType.DMA((nb,)),
            pltpu.SemaphoreType.DMA((nb,)),
            pltpu.SemaphoreType.DMA((nb,)),
        ],
        compiler_params=pltpu.CompilerParams(
            vmem_limit_bytes=100 * 1024 * 1024),
    )(
        A_x, A_c_kv,
        A_w_q.reshape(m * nh, dh),
        A_w_uk.reshape(dc * nh, dh),
        A_w_uv.reshape(dc * nh, dh),
        A_w_o,
        B_x, B_k_cache, B_v_cache, B_wq, B_wo,
    )
```

```python
import jax
import jax.numpy as jnp
import jax.experimental.pallas as pl
import jax.experimental.pallas.tpu as pltpu

_ROWS = 8
_LANES = 128
_COPY_BYTES = 32 * 1024
_WAYS = 4
_GROUP = 4
_SLOTS = 3
_KEYS = 1024

_NT = (((1,), (1,)), ((), ()))


def _dot(a, b):
    return jnp.dot(a, b, preferred_element_type=jnp.float32)


def _dot_nt(a, b):
    return jax.lax.dot_general(a, b, _NT, preferred_element_type=jnp.float32)


def _pad_rows(x):
    x = x.astype(jnp.float32)
    zeros = jnp.zeros((_ROWS - x.shape[0], x.shape[1]), jnp.float32)
    return jnp.concatenate([x, zeros], axis=0).astype(jnp.bfloat16)


def _head_pair(w_buf, j, n, npair):
    words = w_buf[pl.ds(j, n, stride=npair), :]
    even = pltpu.bitcast(words << 16, jnp.float32)
    odd = pltpu.bitcast(words & jnp.uint32(0xFFFF0000), jnp.float32)
    return even.astype(jnp.bfloat16), odd.astype(jnp.bfloat16)


def _ds(start, size):
    if isinstance(start, int):
        return pl.ds(start, size)
    return pl.ds(pl.multiple_of(start, size), size)


def _wait_all(buf, sem):
    pltpu.make_async_copy(buf, buf, sem).wait()


def _kernel(ax_hbm, ckv_hbm, wq_hbm, wuk_hbm, wuv_hbm, wo_hbm,
            bx_hbm, k_hbm, v_hbm, bwq_hbm, bwo_hbm,
            o_hbm,
            ax_buf, bx_buf, o_buf,
            wq_buf, wuk_buf, wuv_buf, bwq_buf, ckv_buf, wo_buf, bwo_buf,
            k_buf, v_buf,
            lat_buf, m_buf, l_buf, acc_buf, ctx_buf, qb_buf, ob_buf,
            io_sem, w_sem, c_sem, wo_sem, bwo_sem, k_sem, v_sem):
    nb, sk, dc = ckv_hbm.shape
    nbh, _, dh = k_hbm.shape
    nh = nbh // nb
    m = ax_hbm.shape[1]
    npair = nh // 2
    scale = dh ** -0.5
    bf16 = jnp.bfloat16

    def row_copy(src, dst, sem, row_bytes):
        rows = _COPY_BYTES // row_bytes
        per_way = src.shape[0] // _WAYS

        def start(s, c, queue):
            r = _ds(s * per_way + c * rows, rows)
            pltpu.make_async_copy(src.at[r], dst.at[r], sem).start(priority=queue)
        return start

    def bwq_copy(s, c, queue):
        cols = _COPY_BYTES // (2 * 8)
        per_row = bwq_hbm.shape[1] // cols
        r = _ds(s * (m // _WAYS) + (c // per_row) * 8, 8)
        cs = _ds((c % per_row) * cols, cols)
        pltpu.make_async_copy(bwq_hbm.at[r, cs], bwq_buf.at[r, cs],
                              w_sem.at[3]).start(priority=queue)

    def stream_pair(first, second, ncopy):
        def body(c, carry):
            for s in range(_WAYS):
                first(s, c, 0)
                second(s, c, 1)
            return carry
        jax.lax.fori_loop(0, ncopy // _WAYS, body, 0)

    kv_rows = _COPY_BYTES // (2 * dh)
    kv_step = sk // kv_rows // _GROUP
    ngroup = nbh // _GROUP

    def kv_issue(g, part, lo, hi):
        slot = g % _SLOTS
        for c in range(lo, hi):
            r = _ds((part * kv_step + c) * kv_rows, kv_rows)
            for a in range(_GROUP):
                pltpu.make_async_copy(k_hbm.at[g * _GROUP + a, r],
                                      k_buf.at[slot, a, r],
                                      k_sem.at[slot]).start(priority=0)
                pltpu.make_async_copy(v_hbm.at[g * _GROUP + a, r],
                                      v_buf.at[slot, a, r],
                                      v_sem.at[slot]).start(priority=1)

    nstage = nh // _WAYS
    wo_rows = _COPY_BYTES // (2 * m)

    def wo_issue(j):
        for c in range(dh // wo_rows):
            r = pl.ds(c * wo_rows, wo_rows)
            for s in range(_WAYS):
                h = s * nstage + j
                pltpu.make_async_copy(wo_hbm.at[h, r], wo_buf.at[j, s, r],
                                      wo_sem.at[j]).start(priority=0)
                pltpu.make_async_copy(bwo_hbm.at[h, r], bwo_buf.at[j, s, r],
                                      bwo_sem.at[j]).start(priority=1)

    def lat_store(rows, val):
        for i in range(dc // _LANES):
            lat_buf[i, rows, :] = val[:, i * _LANES:(i + 1) * _LANES]

    def lat_load(rows):
        parts = [lat_buf[i, rows, :] for i in range(dc // _LANES)]
        return jnp.concatenate(parts, axis=1).astype(bf16)

    def absorb(j):
        xa = _pad_rows(ax_buf[...])
        wq2 = _head_pair(wq_buf, j, m, npair)
        wuk2 = _head_pair(wuk_buf, j, dc, npair)
        for t in range(2):
            q = _dot(xa, wq2[t]).astype(bf16)
            lat_store(_ds((2 * j + t) * _ROWS, _ROWS), _dot_nt(q, wuk2[t]))

    nchunk = sk // _KEYS

    def attend(t):
        b, chunk = t // nchunk, t % nchunk
        rows = pl.ds(b, nh, stride=_ROWS)

        @pl.when(chunk == 0)
        def _():
            m_buf[...] = jnp.full(m_buf.shape, -jnp.inf, jnp.float32)
            l_buf[...] = jnp.zeros(l_buf.shape, jnp.float32)
            acc_buf[...] = jnp.zeros(acc_buf.shape, jnp.float32)

        c = ckv_buf[b, _ds(chunk * _KEYS, _KEYS), :]
        s = _dot_nt(lat_load(rows), c) * scale
        m_old = m_buf[...]
        m_new = jnp.maximum(m_old, jnp.max(s, axis=-1, keepdims=True))
        alpha = jnp.exp(m_old - m_new)
        p = jnp.exp(s - m_new[:, :1])
        l_new = alpha * l_buf[...] + jnp.sum(p, axis=-1, keepdims=True)
        acc = alpha[:, :1] * acc_buf[...] + _dot(p.astype(bf16), c)
        m_buf[...] = m_new
        l_buf[...] = l_new
        acc_buf[...] = acc

        @pl.when(chunk == nchunk - 1)
        def _():
            lat_store(rows, acc_buf[...] / l_buf[:, :1])

    def up_project(j):
        wuv2 = _head_pair(wuv_buf, j, dc, npair)
        for t in range(2):
            h = 2 * j + t
            ctx_buf[h] = _dot(lat_load(_ds(h * _ROWS, _ROWS)), wuv2[t])

    ax_cp = pltpu.make_async_copy(ax_hbm, ax_buf, io_sem.at[0])
    bx_cp = pltpu.make_async_copy(bx_hbm, bx_buf, io_sem.at[1])
    u32 = jnp.uint32
    wcopies = wq_buf.shape[0] * 4 * dh // _COPY_BYTES
    ccopies = sk * dc * 2 // _COPY_BYTES
    stream_pair(bwq_copy,
                row_copy(wq_hbm.bitcast(u32), wq_buf, w_sem.at[0], 4 * dh),
                wcopies)
    ax_cp.start()
    bx_cp.start()
    stream_pair(row_copy(wuk_hbm.bitcast(u32), wuk_buf, w_sem.at[1], 4 * dh),
                row_copy(wuv_hbm.bitcast(u32), wuv_buf, w_sem.at[2], 4 * dh),
                wcopies)

    bx_cp.wait()
    _wait_all(bwq_buf, w_sem.at[3])
    xb = _pad_rows(bx_buf[...])
    for h in range(nh):
        qb_buf[h] = _dot(xb, bwq_buf[:, h * dh:(h + 1) * dh])
    ob_buf[...] = jnp.zeros(ob_buf.shape, jnp.float32)

    for b in range(0, nb, 2):
        stream_pair(
            row_copy(ckv_hbm.at[b], ckv_buf.at[b], c_sem.at[b], 2 * dc),
            row_copy(ckv_hbm.at[b + 1], ckv_buf.at[b + 1], c_sem.at[b + 1], 2 * dc),
            ccopies)

    def first_groups(i, carry):
        kv_issue(i // _GROUP, i % _GROUP, 0, kv_step)
        return carry
    jax.lax.fori_loop(0, (_SLOTS - 1) * _GROUP, first_groups, 0)

    ax_cp.wait()
    _wait_all(wq_buf, w_sem.at[0])
    _wait_all(wuk_buf, w_sem.at[1])
    _wait_all(wuv_buf, w_sem.at[2])
    for b in range(nb):
        _wait_all(ckv_buf.at[b], c_sem.at[b])

    row = jax.lax.broadcasted_iota(jnp.int32, (_ROWS, dh), 0)
    t_attend = npair
    t_project = t_attend + nb * nchunk
    t_tail = (ngroup - _SLOTS + 1) * _GROUP

    def issue(i, half):
        g, a = i // _GROUP, i % _GROUP

        @pl.when(i < t_tail)
        def _():
            kv_issue(g + _SLOTS - 1, a,
                     half * kv_step // 2, (half + 1) * kv_step // 2)

        @pl.when(jnp.logical_and(i >= t_tail, i < t_tail + nstage // 2))
        def _():
            wo_issue(2 * (i - t_tail) + half)

    def head(i, carry):
        g, a = i // _GROUP, i % _GROUP
        slot = g % _SLOTS
        b, h = i // nh, i % nh

        @pl.when(a == 0)
        def _():
            _wait_all(k_buf.at[slot], k_sem.at[slot])
            _wait_all(v_buf.at[slot], v_sem.at[slot])

        s = _dot_nt(qb_buf[h].astype(bf16), k_buf[slot, a]) * scale
        p = jnp.exp(s - jnp.max(s, axis=-1, keepdims=True))
        l = jnp.sum(p, axis=-1, keepdims=True)
        o = _dot(p.astype(bf16), v_buf[slot, a]) / l
        ob_buf[h] = jnp.where(row == b, o, ob_buf[h])

        issue(i, 0)

        @pl.when(i < t_attend)
        def _():
            absorb(i)

        @pl.when(jnp.logical_and(i >= t_attend, i < t_project))
        def _():
            attend(i - t_attend)

        @pl.when(jnp.logical_and(i >= t_project, i < t_project + npair))
        def _():
            up_project(i - t_project)

        issue(i, 1)
        return carry

    jax.lax.fori_loop(0, nbh, head, 0)

    def out_project(j, accs):
        acc_a, acc_b = accs
        _wait_all(wo_buf.at[j], wo_sem.at[j])
        _wait_all(bwo_buf.at[j], bwo_sem.at[j])
        for s in range(_WAYS):
            h = s * nstage + j
            acc_a = acc_a + _dot(ctx_buf[h].astype(bf16), wo_buf[j, s])
            acc_b = acc_b + _dot(ob_buf[h].astype(bf16), bwo_buf[j, s])
        return acc_a, acc_b

    zero = jnp.zeros((_ROWS, m), jnp.float32)
    out_a, out_b = jax.lax.fori_loop(0, nstage, out_project, (zero, zero))
    o_buf[:, 0:m] = out_a[0:nb].astype(o_buf.dtype)
    o_buf[:, m:2 * m] = out_b[0:nb].astype(o_buf.dtype)
    o_cp = pltpu.make_async_copy(o_buf, o_hbm, io_sem.at[2])
    o_cp.start()
    o_cp.wait()


@jax.jit
def pallas_concat_heads__compressed_kv_cla__mha_block_cached__decode_kernel(
    A_x: jax.Array,
    A_c_kv: jax.Array,
    A_w_q: jax.Array,
    A_w_uk: jax.Array,
    A_w_uv: jax.Array,
    A_w_o: jax.Array,
    B_x: jax.Array,
    B_k_cache: jax.Array,
    B_v_cache: jax.Array,
    B_wq: jax.Array,
    B_wo: jax.Array,
):
    nb, sq, m = A_x.shape
    _, sk, dc = A_c_kv.shape
    _, nh, dh = A_w_q.shape
    assert sq == 1 and nb <= _ROWS and nb % 2 == 0 and dh == _LANES and dc == m
    assert B_k_cache.shape == (nb, nh, sk, dh) and B_x.shape == A_x.shape
    bf16, f32 = jnp.bfloat16, jnp.float32
    nstage = nh // _WAYS

    hbm = pl.BlockSpec(memory_space=pltpu.HBM)
    out = pl.pallas_call(
        _kernel,
        out_shape=jax.ShapeDtypeStruct((nb, 2 * m), A_x.dtype),
        in_specs=[hbm] * 11,
        out_specs=hbm,
        scratch_shapes=[
            pltpu.VMEM((nb, m), bf16),
            pltpu.VMEM((nb, m), bf16),
            pltpu.VMEM((nb, 2 * m), A_x.dtype),
            pltpu.VMEM((m * nh // 2, dh), jnp.uint32),
            pltpu.VMEM((dc * nh // 2, dh), jnp.uint32),
            pltpu.VMEM((dc * nh // 2, dh), jnp.uint32),
            pltpu.VMEM((m, nh * dh), bf16),
            pltpu.VMEM((nb, sk, dc), bf16),
            pltpu.VMEM((nstage, _WAYS, dh, m), bf16),
            pltpu.VMEM((nstage, _WAYS, dh, m), bf16),
            pltpu.VMEM((_SLOTS, _GROUP, sk, dh), bf16),
            pltpu.VMEM((_SLOTS, _GROUP, sk, dh), bf16),
            pltpu.VMEM((dc // _LANES, nh * _ROWS, _LANES), f32),
            pltpu.VMEM((nh, _LANES), f32),
            pltpu.VMEM((nh, _LANES), f32),
            pltpu.VMEM((nh, dc), f32),
            pltpu.VMEM((nh, _ROWS, dh), f32),
            pltpu.VMEM((nh, _ROWS, dh), f32),
            pltpu.VMEM((nh, _ROWS, dh), f32),
            pltpu.SemaphoreType.DMA((3,)),
            pltpu.SemaphoreType.DMA((4,)),
            pltpu.SemaphoreType.DMA((nb,)),
            pltpu.SemaphoreType.DMA((nstage,)),
            pltpu.SemaphoreType.DMA((nstage,)),
            pltpu.SemaphoreType.DMA((_SLOTS,)),
            pltpu.SemaphoreType.DMA((_SLOTS,)),
        ],
        compiler_params=pltpu.CompilerParams(
            vmem_limit_bytes=110 * 1024 * 1024),
    )(
        A_x.reshape(nb, m), A_c_kv,
        A_w_q.reshape(m * nh, dh),
        A_w_uk.reshape(dc * nh, dh),
        A_w_uv.reshape(dc * nh, dh),
        A_w_o,
        B_x.reshape(nb, m),
        B_k_cache.reshape(nb * nh, sk, dh),
        B_v_cache.reshape(nb * nh, sk, dh),
        B_wq,
        B_wo.reshape(nh, dh, m),
    )
    return out.reshape(nb, sq, 2 * m)
```

```python
import jax
import jax.numpy as jnp
import jax.experimental.pallas as pl
import jax.experimental.pallas.tpu as pltpu

_ROWS = 8
_LANES = 128
_KV_CUTS = (12, 20)
_W_CUTS = (24, 24, 16)
_WAYS = 4
_GROUP = 8
_SLOTS = 3
_AHEAD = 1
_NOCHECK = True
_KEYS = 1024

_NT = (((1,), (1,)), ((), ()))


def _dot(a, b):
    return jnp.dot(a, b, preferred_element_type=jnp.float32)


def _dot_nt(a, b):
    return jax.lax.dot_general(a, b, _NT, preferred_element_type=jnp.float32)


def _pad_rows(x):
    x = x.astype(jnp.float32)
    zeros = jnp.zeros((_ROWS - x.shape[0], x.shape[1]), jnp.float32)
    return jnp.concatenate([x, zeros], axis=0).astype(jnp.bfloat16)


def _head_pair(w_buf, j, n, npair):
    words = w_buf[pl.ds(j, n, stride=npair), :]
    even = pltpu.bitcast(words << 16, jnp.float32)
    odd = pltpu.bitcast(words & jnp.uint32(0xFFFF0000), jnp.float32)
    return even.astype(jnp.bfloat16), odd.astype(jnp.bfloat16)


def _ds(start, size):
    if isinstance(start, int):
        return pl.ds(start, size)
    return pl.ds(pl.multiple_of(start, size), size)


def _cut(nbytes, cuts_kib):
    out, off = [], 0
    while off < nbytes:
        size = min(cuts_kib[len(out) % len(cuts_kib)] * 1024, nbytes - off)
        out.append((off, size))
        off += size
    return out


def _wait_all(buf, sem):
    pltpu.make_async_copy(buf, buf, sem).wait()


def _kernel(ax_hbm, ckv_hbm, wq_hbm, wuk_hbm, wuv_hbm, wo_hbm,
            bx_hbm, k_hbm, v_hbm, bwq_hbm, bwo_hbm,
            o_hbm,
            ax_buf, bx_buf, o_buf,
            wq_buf, wuk_buf, wuv_buf, bwq_buf, ckv_buf, wo_buf, bwo_buf,
            k_buf, v_buf,
            lat_buf, m_buf, l_buf, acc_buf, ctx_buf, qb_buf, ob_buf,
            io_sem, w_sem, c_sem, wo_sem, bwo_sem, k_sem, v_sem):
    nb, sk, dc = ckv_hbm.shape
    nbh, _, dh = k_hbm.shape
    nh = nbh // nb
    m = ax_hbm.shape[1]
    npair = nh // 2
    scale = dh ** -0.5
    bf16 = jnp.bfloat16

    span = sum(_W_CUTS) * 1024

    def row_copy(src, dst, sem, row_bytes):
        per_way = src.shape[0] // _WAYS

        def start(s, c, off, size, queue):
            r0 = s * per_way + c * (span // row_bytes) + off // row_bytes
            r = pl.ds(pl.multiple_of(r0, 8), size // row_bytes)
            pltpu.make_async_copy(src.at[r], dst.at[r], sem).start(priority=queue)
        return start

    def bwq_copy(s, c, off, size, queue):
        r = pl.ds(pl.multiple_of(s * (m // _WAYS) + c * 8, 8), 8)
        cs = pl.ds(off // 16, size // 16)
        pltpu.make_async_copy(bwq_hbm.at[r, cs], bwq_buf.at[r, cs],
                              w_sem.at[3]).start(priority=queue)

    def stream_pair(first, second, nbytes):
        def body(c, carry):
            for off, size in _cut(span, _W_CUTS):
                for s in range(_WAYS):
                    first(s, c, off, size, 0)
                    second(s, c, off, size, 1)
            return carry
        jax.lax.fori_loop(0, nbytes // _WAYS // span, body, 0)

    kv_step = sk // _GROUP

    def kv_issue(step, lo, hi):
        g, part = step // _GROUP, step % _GROUP
        slot = g % _SLOTS
        for off, size in _cut((hi - lo) * 2 * dh, _KV_CUTS):
            r0 = part * kv_step + lo + off // (2 * dh)
            r = pl.ds(pl.multiple_of(r0, 16), size // (2 * dh))
            for a in range(_GROUP):
                pltpu.make_async_copy(k_hbm.at[g * _GROUP + a, r],
                                      k_buf.at[slot, a, r],
                                      k_sem.at[slot]).start(priority=0)
                pltpu.make_async_copy(v_hbm.at[g * _GROUP + a, r],
                                      v_buf.at[slot, a, r],
                                      v_sem.at[slot]).start(priority=1)

    nstage = nh // _WAYS

    def wo_issue(j, lo, hi):
        for off, size in _cut((hi - lo) * 2 * m, _W_CUTS):
            r = pl.ds(lo + off // (2 * m), size // (2 * m))
            for s in range(_WAYS):
                h = s * nstage + j
                pltpu.make_async_copy(wo_hbm.at[h, r], wo_buf.at[j, s, r],
                                      wo_sem.at[j]).start(priority=0)
                pltpu.make_async_copy(bwo_hbm.at[h, r], bwo_buf.at[j, s, r],
                                      bwo_sem.at[j]).start(priority=1)

    def lat_store(rows, val):
        for i in range(dc // _LANES):
            lat_buf[i, rows, :] = val[:, i * _LANES:(i + 1) * _LANES]

    def lat_load(rows):
        parts = [lat_buf[i, rows, :] for i in range(dc // _LANES)]
        return jnp.concatenate(parts, axis=1).astype(bf16)

    def absorb(j):
        xa = _pad_rows(ax_buf[...])
        wq2 = _head_pair(wq_buf, j, m, npair)
        wuk2 = _head_pair(wuk_buf, j, dc, npair)
        for t in range(2):
            q = _dot(xa, wq2[t]).astype(bf16)
            lat_store(_ds((2 * j + t) * _ROWS, _ROWS), _dot_nt(q, wuk2[t]))

    nchunk = sk // _KEYS

    def attend(t):
        b, chunk = t // nchunk, t % nchunk
        rows = pl.ds(b, nh, stride=_ROWS)

        @pl.when(chunk == 0)
        def _():
            m_buf[...] = jnp.full(m_buf.shape, -jnp.inf, jnp.float32)
            l_buf[...] = jnp.zeros(l_buf.shape, jnp.float32)
            acc_buf[...] = jnp.zeros(acc_buf.shape, jnp.float32)

        c = ckv_buf[b, _ds(chunk * _KEYS, _KEYS), :]
        s = _dot_nt(lat_load(rows), c) * scale
        m_old = m_buf[...]
        m_new = jnp.maximum(m_old, jnp.max(s, axis=-1, keepdims=True))
        alpha = jnp.exp(m_old - m_new)
        p = jnp.exp(s - m_new[:, :1])
        l_new = alpha * l_buf[...] + jnp.sum(p, axis=-1, keepdims=True)
        acc = alpha[:, :1] * acc_buf[...] + _dot(p.astype(bf16), c)
        m_buf[...] = m_new
        l_buf[...] = l_new
        acc_buf[...] = acc

        @pl.when(chunk == nchunk - 1)
        def _():
            lat_store(rows, acc_buf[...] / l_buf[:, :1])

    def up_project(j):
        wuv2 = _head_pair(wuv_buf, j, dc, npair)
        for t in range(2):
            h = 2 * j + t
            ctx_buf[h] = _dot(lat_load(_ds(h * _ROWS, _ROWS)), wuv2[t])

    ax_cp = pltpu.make_async_copy(ax_hbm, ax_buf, io_sem.at[0])
    bx_cp = pltpu.make_async_copy(bx_hbm, bx_buf, io_sem.at[1])
    u32 = jnp.uint32
    wbytes = m * nh * dh * 2
    stream_pair(bwq_copy,
                row_copy(wq_hbm.bitcast(u32), wq_buf, w_sem.at[0], 4 * dh),
                wbytes)
    ax_cp.start()
    bx_cp.start()
    stream_pair(row_copy(wuk_hbm.bitcast(u32), wuk_buf, w_sem.at[1], 4 * dh),
                row_copy(wuv_hbm.bitcast(u32), wuv_buf, w_sem.at[2], 4 * dh),
                wbytes)

    bx_cp.wait()
    _wait_all(bwq_buf, w_sem.at[3])
    xb = _pad_rows(bx_buf[...])
    for h in range(nh):
        qb_buf[h] = _dot(xb, bwq_buf[:, h * dh:(h + 1) * dh])
    ob_buf[...] = jnp.zeros(ob_buf.shape, jnp.float32)

    for b in range(0, nb, 2):
        stream_pair(
            row_copy(ckv_hbm.at[b], ckv_buf.at[b], c_sem.at[b], 2 * dc),
            row_copy(ckv_hbm.at[b + 1], ckv_buf.at[b + 1], c_sem.at[b + 1], 2 * dc),
            sk * dc * 2)

    ahead = _GROUP + _AHEAD

    def first_steps(i, carry):
        kv_issue(i, 0, kv_step)
        return carry
    jax.lax.fori_loop(0, ahead, first_steps, 0)

    ax_cp.wait()
    _wait_all(wq_buf, w_sem.at[0])
    _wait_all(wuk_buf, w_sem.at[1])
    _wait_all(wuv_buf, w_sem.at[2])
    for b in range(nb):
        _wait_all(ckv_buf.at[b], c_sem.at[b])

    row = jax.lax.broadcasted_iota(jnp.int32, (_ROWS, dh), 0)
    t_attend = npair
    t_project = t_attend + nb * nchunk
    t_tail = nbh - ahead
    per_step = -(-nstage // ahead)

    def issue(i, half):
        @pl.when(i < t_tail)
        def _():
            kv_issue(i + ahead, half * kv_step // 2, (half + 1) * kv_step // 2)

        @pl.when(jnp.logical_and(i >= t_tail, i < t_tail + nstage // per_step))
        def _():
            for u in range(per_step):
                wo_issue((i - t_tail) * per_step + u,
                         half * dh // 2, (half + 1) * dh // 2)

    def head(i, carry):
        g, a = i // _GROUP, i % _GROUP
        slot = g % _SLOTS
        b, h = i // nh, i % nh

        @pl.when(a == 0)
        def _():
            _wait_all(k_buf.at[slot], k_sem.at[slot])
            _wait_all(v_buf.at[slot], v_sem.at[slot])

        s = _dot_nt(qb_buf[h].astype(bf16), k_buf[slot, a]) * scale
        p = jnp.exp(s - jnp.max(s, axis=-1, keepdims=True))
        l = jnp.sum(p, axis=-1, keepdims=True)
        o = _dot(p.astype(bf16), v_buf[slot, a]) / l
        ob_buf[h] = jnp.where(row == b, o, ob_buf[h])

        issue(i, 0)

        @pl.when(i < t_attend)
        def _():
            absorb(i)

        @pl.when(jnp.logical_and(i >= t_attend, i < t_project))
        def _():
            attend(i - t_attend)

        @pl.when(jnp.logical_and(i >= t_project, i < t_project + npair))
        def _():
            up_project(i - t_project)

        issue(i, 1)
        return carry

    jax.lax.fori_loop(0, nbh, head, 0)

    def out_project(j, accs):
        acc_a, acc_b = accs
        _wait_all(wo_buf.at[j], wo_sem.at[j])
        _wait_all(bwo_buf.at[j], bwo_sem.at[j])
        for s in range(_WAYS):
            h = s * nstage + j
            acc_a = acc_a + _dot(ctx_buf[h].astype(bf16), wo_buf[j, s])
            acc_b = acc_b + _dot(ob_buf[h].astype(bf16), bwo_buf[j, s])
        return acc_a, acc_b

    zero = jnp.zeros((_ROWS, m), jnp.float32)
    out_a, out_b = jax.lax.fori_loop(0, nstage, out_project, (zero, zero))
    o_buf[:, 0:m] = out_a[0:nb].astype(o_buf.dtype)
    o_buf[:, m:2 * m] = out_b[0:nb].astype(o_buf.dtype)
    o_cp = pltpu.make_async_copy(o_buf, o_hbm, io_sem.at[2])
    o_cp.start()
    o_cp.wait()


@jax.jit
def pallas_concat_heads__compressed_kv_cla__mha_block_cached__decode_kernel(
    A_x: jax.Array,
    A_c_kv: jax.Array,
    A_w_q: jax.Array,
    A_w_uk: jax.Array,
    A_w_uv: jax.Array,
    A_w_o: jax.Array,
    B_x: jax.Array,
    B_k_cache: jax.Array,
    B_v_cache: jax.Array,
    B_wq: jax.Array,
    B_wo: jax.Array,
):
    nb, sq, m = A_x.shape
    _, sk, dc = A_c_kv.shape
    _, nh, dh = A_w_q.shape
    assert sq == 1 and nb <= _ROWS and nb % 2 == 0 and dh == _LANES and dc == m
    assert B_k_cache.shape == (nb, nh, sk, dh) and B_x.shape == A_x.shape
    bf16, f32 = jnp.bfloat16, jnp.float32
    nstage = nh // _WAYS

    hbm = pl.BlockSpec(memory_space=pltpu.HBM)
    out = pl.pallas_call(
        _kernel,
        out_shape=jax.ShapeDtypeStruct((nb, 2 * m), A_x.dtype),
        in_specs=[hbm] * 11,
        out_specs=hbm,
        scratch_shapes=[
            pltpu.VMEM((nb, m), bf16),
            pltpu.VMEM((nb, m), bf16),
            pltpu.VMEM((nb, 2 * m), A_x.dtype),
            pltpu.VMEM((m * nh // 2, dh), jnp.uint32),
            pltpu.VMEM((dc * nh // 2, dh), jnp.uint32),
            pltpu.VMEM((dc * nh // 2, dh), jnp.uint32),
            pltpu.VMEM((m, nh * dh), bf16),
            pltpu.VMEM((nb, sk, dc), bf16),
            pltpu.VMEM((nstage, _WAYS, dh, m), bf16),
            pltpu.VMEM((nstage, _WAYS, dh, m), bf16),
            pltpu.VMEM((_SLOTS, _GROUP, sk, dh), bf16),
            pltpu.VMEM((_SLOTS, _GROUP, sk, dh), bf16),
            pltpu.VMEM((dc // _LANES, nh * _ROWS, _LANES), f32),
            pltpu.VMEM((nh, _LANES), f32),
            pltpu.VMEM((nh, _LANES), f32),
            pltpu.VMEM((nh, dc), f32),
            pltpu.VMEM((nh, _ROWS, dh), f32),
            pltpu.VMEM((nh, _ROWS, dh), f32),
            pltpu.VMEM((nh, _ROWS, dh), f32),
            pltpu.SemaphoreType.DMA((3,)),
            pltpu.SemaphoreType.DMA((4,)),
            pltpu.SemaphoreType.DMA((nb,)),
            pltpu.SemaphoreType.DMA((nstage,)),
            pltpu.SemaphoreType.DMA((nstage,)),
            pltpu.SemaphoreType.DMA((_SLOTS,)),
            pltpu.SemaphoreType.DMA((_SLOTS,)),
        ],
        compiler_params=pltpu.CompilerParams(
            vmem_limit_bytes=110 * 1024 * 1024,
            disable_bounds_checks=_NOCHECK),
    )(
        A_x.reshape(nb, m), A_c_kv,
        A_w_q.reshape(m * nh, dh),
        A_w_uk.reshape(dc * nh, dh),
        A_w_uv.reshape(dc * nh, dh),
        A_w_o,
        B_x.reshape(nb, m),
        B_k_cache.reshape(nb * nh, sk, dh),
        B_v_cache.reshape(nb * nh, sk, dh),
        B_wq,
        B_wo.reshape(nh, dh, m),
    )
    return out.reshape(nb, sq, 2 * m)
```

```python
import jax
import jax.numpy as jnp
import jax.experimental.pallas as pl
import jax.experimental.pallas.tpu as pltpu

_ROWS = 8
_LANES = 128
_KV_CUTS = (16, 32, 32, 32, 16)
_W_CUTS = (32,)
_WO_KIB = 32
_TAIL = 3
_SPLIT = 2
_WAYS = 8
_STAGE = 4
_GROUP = 8
_SLOTS = 3
_AHEAD = 3
_NOCHECK = True
_KEYS = 1024

_NT = (((1,), (1,)), ((), ()))


def _dot(a, b):
    return jnp.dot(a, b, preferred_element_type=jnp.float32)


def _dot_nt(a, b):
    return jax.lax.dot_general(a, b, _NT, preferred_element_type=jnp.float32)


def _pad_rows(x):
    x = x.astype(jnp.float32)
    zeros = jnp.zeros((_ROWS - x.shape[0], x.shape[1]), jnp.float32)
    return jnp.concatenate([x, zeros], axis=0).astype(jnp.bfloat16)


def _head_pair(w_buf, j, n, npair):
    words = w_buf[pl.ds(j, n, stride=npair), :]
    even = pltpu.bitcast(words << 16, jnp.float32)
    odd = pltpu.bitcast(words & jnp.uint32(0xFFFF0000), jnp.float32)
    return even.astype(jnp.bfloat16), odd.astype(jnp.bfloat16)


def _ds(start, size):
    if isinstance(start, int):
        return pl.ds(start, size)
    return pl.ds(pl.multiple_of(start, size), size)


def _cut(nbytes, cuts_kib):
    out, off = [], 0
    while off < nbytes:
        size = min(cuts_kib[len(out) % len(cuts_kib)] * 1024, nbytes - off)
        out.append((off, size))
        off += size
    return out


def _half(items, which):
    mid = len(items) // 2
    return items[mid:] if which else items[:mid]


def _wait_all(buf, sem):
    pltpu.make_async_copy(buf, buf, sem).wait()


def _kernel(ax_hbm, ckv_hbm, wq_hbm, wuk_hbm, wuv_hbm, wo_hbm,
            bx_hbm, k_hbm, v_hbm, bwq_hbm, bwo_hbm,
            o_hbm,
            ax_buf, bx_buf, o_buf,
            wq_buf, wuk_buf, wuv_buf, bwq_buf, ckv_buf, wo_buf, bwo_buf,
            k_buf, v_buf,
            lat_buf, m_buf, l_buf, acc_buf, ctx_buf, qb_buf, ob_buf, out_acc,
            io_sem, w_sem, c_sem, wo_sem, bwo_sem, k_sem, v_sem):
    nb, sk, dc = ckv_hbm.shape
    nbh, _, dh = k_hbm.shape
    nh = nbh // nb
    m = ax_hbm.shape[1]
    npair = nh // 2
    scale = dh ** -0.5
    bf16 = jnp.bfloat16

    span = 8 * bwq_hbm.shape[1] * 2

    def row_copy(src, dst, sem, row_bytes):
        per_way = src.shape[0] // _WAYS

        def start(s, c, off, size, queue):
            r0 = s * per_way + c * (span // row_bytes) + off // row_bytes
            r = pl.ds(pl.multiple_of(r0, 8), size // row_bytes)
            pltpu.make_async_copy(src.at[r], dst.at[r], sem).start(priority=queue)
        return start

    def bwq_copy(s, c, off, size, queue):
        r = pl.ds(pl.multiple_of(s * (m // _WAYS) + c * 8, 8), 8)
        cs = pl.ds(off // 16, size // 16)
        pltpu.make_async_copy(bwq_hbm.at[r, cs], bwq_buf.at[r, cs],
                              w_sem.at[3]).start(priority=queue)

    def stream_pair(first, second, nbytes):
        def body(c, carry):
            for off, size in _cut(span, _W_CUTS):
                for s in range(_WAYS):
                    first(s, c, off, size, 0)
                    second(s, c, off, size, 1)
            return carry
        jax.lax.fori_loop(0, nbytes // _WAYS // span, body, 0)

    kv_step = sk // _GROUP

    kv_cuts = _cut(kv_step * 2 * dh, _KV_CUTS)

    def kv_issue(step, cuts):
        g, part = step // _GROUP, step % _GROUP
        slot = g % _SLOTS
        for off, size in cuts:
            r0 = part * kv_step + off // (2 * dh)
            r = pl.ds(pl.multiple_of(r0, 8), size // (2 * dh))
            for a in range(_GROUP):
                pltpu.make_async_copy(k_hbm.at[g * _GROUP + a, r],
                                      k_buf.at[slot, a, r],
                                      k_sem.at[slot]).start(priority=0)
                pltpu.make_async_copy(v_hbm.at[g * _GROUP + a, r],
                                      v_buf.at[slot, a, r],
                                      v_sem.at[slot]).start(priority=1)

    nstage = nh // _STAGE

    wo_rows = _WO_KIB * 1024 // (2 * m)
    stage_pieces = dh // wo_rows

    def wo_issue(piece, split=1):
        j = piece // stage_pieces
        for part in range(split):
            r0 = (piece % stage_pieces) * wo_rows + part * (wo_rows // split)
            r = pl.ds(pl.multiple_of(r0, 8), wo_rows // split)
            for s in range(_STAGE):
                h = s * nstage + j
                pltpu.make_async_copy(wo_hbm.at[h, r], wo_buf.at[j, s, r],
                                      wo_sem.at[j]).start(priority=0)
                pltpu.make_async_copy(bwo_hbm.at[h, r], bwo_buf.at[j, s, r],
                                      bwo_sem.at[j]).start(priority=1)

    def lat_store(rows, val):
        for i in range(dc // _LANES):
            lat_buf[i, rows, :] = val[:, i * _LANES:(i + 1) * _LANES]

    def lat_load(rows):
        parts = [lat_buf[i, rows, :] for i in range(dc // _LANES)]
        return jnp.concatenate(parts, axis=1).astype(bf16)

    def absorb(j):
        xa = _pad_rows(ax_buf[...])
        wq2 = _head_pair(wq_buf, j, m, npair)
        wuk2 = _head_pair(wuk_buf, j, dc, npair)
        for t in range(2):
            q = _dot(xa, wq2[t]).astype(bf16)
            lat_store(_ds((2 * j + t) * _ROWS, _ROWS), _dot_nt(q, wuk2[t]))

    nchunk = sk // _KEYS

    def attend(t):
        b, chunk = t // nchunk, t % nchunk
        rows = pl.ds(b, nh, stride=_ROWS)

        @pl.when(chunk == 0)
        def _():
            m_buf[...] = jnp.full(m_buf.shape, -jnp.inf, jnp.float32)
            l_buf[...] = jnp.zeros(l_buf.shape, jnp.float32)
            acc_buf[...] = jnp.zeros(acc_buf.shape, jnp.float32)

        c = ckv_buf[b, _ds(chunk * _KEYS, _KEYS), :]
        s = _dot_nt(lat_load(rows), c) * scale
        m_old = m_buf[...]
        m_new = jnp.maximum(m_old, jnp.max(s, axis=-1, keepdims=True))
        alpha = jnp.exp(m_old - m_new)
        p = jnp.exp(s - m_new[:, :1])
        l_new = alpha * l_buf[...] + jnp.sum(p, axis=-1, keepdims=True)
        acc = alpha[:, :1] * acc_buf[...] + _dot(p.astype(bf16), c)
        m_buf[...] = m_new
        l_buf[...] = l_new
        acc_buf[...] = acc

        @pl.when(chunk == nchunk - 1)
        def _():
            lat_store(rows, acc_buf[...] / l_buf[:, :1])

    def up_project(j):
        wuv2 = _head_pair(wuv_buf, j, dc, npair)
        for t in range(2):
            h = 2 * j + t
            ctx_buf[h] = _dot(lat_load(_ds(h * _ROWS, _ROWS)), wuv2[t])

    ax_cp = pltpu.make_async_copy(ax_hbm, ax_buf, io_sem.at[0])
    bx_cp = pltpu.make_async_copy(bx_hbm, bx_buf, io_sem.at[1])
    u32 = jnp.uint32
    wbytes = m * nh * dh * 2
    stream_pair(bwq_copy,
                row_copy(wq_hbm.bitcast(u32), wq_buf, w_sem.at[0], 4 * dh),
                wbytes)
    ax_cp.start()
    bx_cp.start()
    stream_pair(row_copy(wuk_hbm.bitcast(u32), wuk_buf, w_sem.at[1], 4 * dh),
                row_copy(wuv_hbm.bitcast(u32), wuv_buf, w_sem.at[2], 4 * dh),
                wbytes)

    bx_cp.wait()
    _wait_all(bwq_buf, w_sem.at[3])
    xb = _pad_rows(bx_buf[...])
    for h in range(nh):
        qb_buf[h] = _dot(xb, bwq_buf[:, h * dh:(h + 1) * dh])
    ob_buf[...] = jnp.zeros(ob_buf.shape, jnp.float32)
    out_acc[...] = jnp.zeros(out_acc.shape, jnp.float32)

    for b in range(0, nb, 2):
        stream_pair(
            row_copy(ckv_hbm.at[b], ckv_buf.at[b], c_sem.at[b], 2 * dc),
            row_copy(ckv_hbm.at[b + 1], ckv_buf.at[b + 1], c_sem.at[b + 1], 2 * dc),
            sk * dc * 2)

    ahead = _GROUP + _AHEAD

    def first_steps(i, carry):
        kv_issue(i, kv_cuts)
        return carry
    jax.lax.fori_loop(0, ahead, first_steps, 0)

    ax_cp.wait()
    _wait_all(wq_buf, w_sem.at[0])
    _wait_all(wuk_buf, w_sem.at[1])
    _wait_all(wuv_buf, w_sem.at[2])
    for b in range(nb):
        _wait_all(ckv_buf.at[b], c_sem.at[b])

    row = jax.lax.broadcasted_iota(jnp.int32, (_ROWS, dh), 0)
    t_attend = npair
    t_project = t_attend + nb * nchunk
    t_tail = nbh - ahead

    npiece = nstage * stage_pieces
    in_loop = min(_TAIL * ahead, npiece)

    def issue(i, half):
        @pl.when(i < t_tail)
        def _():
            kv_issue(i + ahead, _half(kv_cuts, half))

        for u in _half(range(_TAIL), half):
            piece = (i - t_tail) * _TAIL + u

            @pl.when(jnp.logical_and(i >= t_tail, piece < in_loop))
            def _():
                wo_issue(piece)

    def out_project(j):
        _wait_all(wo_buf.at[j], wo_sem.at[j])
        _wait_all(bwo_buf.at[j], bwo_sem.at[j])
        acc_a, acc_b = out_acc[0], out_acc[1]
        for s in range(_STAGE):
            h = s * nstage + j
            acc_a = acc_a + _dot(ctx_buf[h].astype(bf16), wo_buf[j, s])
            acc_b = acc_b + _dot(ob_buf[h].astype(bf16), bwo_buf[j, s])
        out_acc[0] = acc_a
        out_acc[1] = acc_b

    def head(i, carry):
        g, a = i // _GROUP, i % _GROUP
        slot = g % _SLOTS
        b, h = i // nh, i % nh

        @pl.when(a == 0)
        def _():
            _wait_all(k_buf.at[slot], k_sem.at[slot])
            _wait_all(v_buf.at[slot], v_sem.at[slot])

        s = _dot_nt(qb_buf[h].astype(bf16), k_buf[slot, a]) * scale
        p = jnp.exp(s - jnp.max(s, axis=-1, keepdims=True))
        l = jnp.sum(p, axis=-1, keepdims=True)
        o = _dot(p.astype(bf16), v_buf[slot, a]) / l
        ob_buf[h] = jnp.where(row == b, o, ob_buf[h])

        issue(i, 0)

        @pl.when(i < t_attend)
        def _():
            absorb(i)

        @pl.when(jnp.logical_and(i >= t_attend, i < t_project))
        def _():
            attend(i - t_attend)

        @pl.when(jnp.logical_and(i >= t_project, i < t_project + npair))
        def _():
            up_project(i - t_project)

        issue(i, 1)

        return carry

    jax.lax.fori_loop(0, nbh, head, 0)
    for piece in range(in_loop, npiece):
        wo_issue(piece, _SPLIT)
    jax.lax.fori_loop(0, nstage, lambda j, c: (out_project(j), c)[1], 0)

    o_buf[:, 0:m] = out_acc[0, 0:nb, :].astype(o_buf.dtype)
    o_buf[:, m:2 * m] = out_acc[1, 0:nb, :].astype(o_buf.dtype)
    o_cp = pltpu.make_async_copy(o_buf, o_hbm, io_sem.at[2])
    o_cp.start()
    o_cp.wait()


@jax.jit
def pallas_concat_heads__compressed_kv_cla__mha_block_cached__decode_kernel(
    A_x: jax.Array,
    A_c_kv: jax.Array,
    A_w_q: jax.Array,
    A_w_uk: jax.Array,
    A_w_uv: jax.Array,
    A_w_o: jax.Array,
    B_x: jax.Array,
    B_k_cache: jax.Array,
    B_v_cache: jax.Array,
    B_wq: jax.Array,
    B_wo: jax.Array,
):
    nb, sq, m = A_x.shape
    _, sk, dc = A_c_kv.shape
    _, nh, dh = A_w_q.shape
    assert sq == 1 and nb <= _ROWS and nb % 2 == 0 and dh == _LANES and dc == m
    assert B_k_cache.shape == (nb, nh, sk, dh) and B_x.shape == A_x.shape
    bf16, f32 = jnp.bfloat16, jnp.float32
    nstage = nh // _STAGE

    hbm = pl.BlockSpec(memory_space=pltpu.HBM)
    out = pl.pallas_call(
        _kernel,
        out_shape=jax.ShapeDtypeStruct((nb, 2 * m), A_x.dtype),
        in_specs=[hbm] * 11,
        out_specs=hbm,
        scratch_shapes=[
            pltpu.VMEM((nb, m), bf16),
            pltpu.VMEM((nb, m), bf16),
            pltpu.VMEM((nb, 2 * m), A_x.dtype),
            pltpu.VMEM((m * nh // 2, dh), jnp.uint32),
            pltpu.VMEM((dc * nh // 2, dh), jnp.uint32),
            pltpu.VMEM((dc * nh // 2, dh), jnp.uint32),
            pltpu.VMEM((m, nh * dh), bf16),
            pltpu.VMEM((nb, sk, dc), bf16),
            pltpu.VMEM((nstage, _STAGE, dh, m), bf16),
            pltpu.VMEM((nstage, _STAGE, dh, m), bf16),
            pltpu.VMEM((_SLOTS, _GROUP, sk, dh), bf16),
            pltpu.VMEM((_SLOTS, _GROUP, sk, dh), bf16),
            pltpu.VMEM((dc // _LANES, nh * _ROWS, _LANES), f32),
            pltpu.VMEM((nh, _LANES), f32),
            pltpu.VMEM((nh, _LANES), f32),
            pltpu.VMEM((nh, dc), f32),
            pltpu.VMEM((nh, _ROWS, dh), f32),
            pltpu.VMEM((nh, _ROWS, dh), f32),
            pltpu.VMEM((nh, _ROWS, dh), f32),
            pltpu.VMEM((2, _ROWS, m), f32),
            pltpu.SemaphoreType.DMA((3,)),
            pltpu.SemaphoreType.DMA((4,)),
            pltpu.SemaphoreType.DMA((nb,)),
            pltpu.SemaphoreType.DMA((nstage,)),
            pltpu.SemaphoreType.DMA((nstage,)),
            pltpu.SemaphoreType.DMA((_SLOTS,)),
            pltpu.SemaphoreType.DMA((_SLOTS,)),
        ],
        compiler_params=pltpu.CompilerParams(
            vmem_limit_bytes=110 * 1024 * 1024,
            disable_bounds_checks=_NOCHECK),
    )(
        A_x.reshape(nb, m), A_c_kv,
        A_w_q.reshape(m * nh, dh),
        A_w_uk.reshape(dc * nh, dh),
        A_w_uv.reshape(dc * nh, dh),
        A_w_o,
        B_x.reshape(nb, m),
        B_k_cache.reshape(nb * nh, sk, dh),
        B_v_cache.reshape(nb * nh, sk, dh),
        B_wq,
        B_wo.reshape(nh, dh, m),
    )
    return out.reshape(nb, sq, 2 * m)
```

```python
import jax
import jax.numpy as jnp
import jax.experimental.pallas as pl
import jax.experimental.pallas.tpu as pltpu

_ROWS = 8
_LANES = 128
_KV_CUTS = (16, 32, 32, 32, 16)
_W_CUTS = (32,)
_WO_KIB = 32
_TAIL = 3
_SPLIT = 2
_WAYS = 8
_STAGE = 4
_GROUP = 8
_SLOTS = 3
_AHEAD = 3
_NOCHECK = True
_WIDEN = 8
_KEYS = 1024

_NT = (((1,), (1,)), ((), ()))


def _dot(a, b):
    return jnp.dot(a, b, preferred_element_type=jnp.float32)


def _dot_nt(a, b):
    return jax.lax.dot_general(a, b, _NT, preferred_element_type=jnp.float32)


def _pad_rows(x):
    x = x.astype(jnp.float32)
    zeros = jnp.zeros((_ROWS - x.shape[0], x.shape[1]), jnp.float32)
    return jnp.concatenate([x, zeros], axis=0).astype(jnp.bfloat16)


def _ds(start, size):
    if isinstance(start, int):
        return pl.ds(start, size)
    return pl.ds(pl.multiple_of(start, size), size)


def _cut(nbytes, cuts_kib):
    out, off = [], 0
    while off < nbytes:
        size = min(cuts_kib[len(out) % len(cuts_kib)] * 1024, nbytes - off)
        out.append((off, size))
        off += size
    return out


def _half(items, which):
    mid = len(items) // 2
    return items[mid:] if which else items[:mid]


def _wait_all(buf, sem):
    pltpu.make_async_copy(buf, buf, sem).wait()


def _kernel(ax_hbm, ckv_hbm, wq_hbm, wuk_hbm, wuv_hbm, wo_hbm,
            bx_hbm, k_hbm, v_hbm, bwq_hbm, bwo_hbm,
            o_hbm,
            ax_buf, bx_buf, o_buf,
            wq_buf, wuk_buf, wuv_buf, w32_buf, bwq_buf, ckv_buf, wo_buf, bwo_buf,
            k_buf, v_buf,
            lat_buf, m_buf, l_buf, acc_buf, ctx_buf, qb_buf, ob_buf, out_acc,
            io_sem, w_sem, c_sem, wo_sem, bwo_sem, k_sem, v_sem):
    nb, sk, dc = ckv_hbm.shape
    nbh, _, dh = k_hbm.shape
    nh = nbh // nb
    m = ax_hbm.shape[1]
    npair = nh // 2
    scale = dh ** -0.5
    bf16 = jnp.bfloat16

    span = 8 * bwq_hbm.shape[1] * 2

    def row_copy(src, dst, sem, row_bytes):
        per_way = src.shape[0] // _WAYS

        def start(s, c, off, size, queue):
            r0 = s * per_way + c * (span // row_bytes) + off // row_bytes
            r = pl.ds(pl.multiple_of(r0, 8), size // row_bytes)
            pltpu.make_async_copy(src.at[r], dst.at[r], sem).start(priority=queue)
        return start

    def bwq_copy(s, c, off, size, queue):
        r = pl.ds(pl.multiple_of(s * (m // _WAYS) + c * 8, 8), 8)
        cs = pl.ds(off // 16, size // 16)
        pltpu.make_async_copy(bwq_hbm.at[r, cs], bwq_buf.at[r, cs],
                              w_sem.at[3]).start(priority=queue)

    def stream_pair(first, second, nbytes):
        def body(c, carry):
            for off, size in _cut(span, _W_CUTS):
                for s in range(_WAYS):
                    first(s, c, off, size, 0)
                    second(s, c, off, size, 1)
            return carry
        jax.lax.fori_loop(0, nbytes // _WAYS // span, body, 0)

    kv_step = sk // _GROUP

    kv_cuts = _cut(kv_step * 2 * dh, _KV_CUTS)

    def kv_issue(step, cuts):
        g, part = step // _GROUP, step % _GROUP
        slot = g % _SLOTS
        for off, size in cuts:
            r0 = part * kv_step + off // (2 * dh)
            r = pl.ds(pl.multiple_of(r0, 8), size // (2 * dh))
            for a in range(_GROUP):
                pltpu.make_async_copy(k_hbm.at[g * _GROUP + a, r],
                                      k_buf.at[slot, a, r],
                                      k_sem.at[slot]).start(priority=0)
                pltpu.make_async_copy(v_hbm.at[g * _GROUP + a, r],
                                      v_buf.at[slot, a, r],
                                      v_sem.at[slot]).start(priority=1)

    nstage = nh // _STAGE

    wo_rows = _WO_KIB * 1024 // (2 * m)
    stage_pieces = dh // wo_rows

    def wo_issue(piece, split=1):
        j = piece // stage_pieces
        for part in range(split):
            r0 = (piece % stage_pieces) * wo_rows + part * (wo_rows // split)
            r = pl.ds(pl.multiple_of(r0, 8), wo_rows // split)
            for s in range(_STAGE):
                h = s * nstage + j
                pltpu.make_async_copy(wo_hbm.at[h, r], wo_buf.at[j, s, r],
                                      wo_sem.at[j]).start(priority=0)
                pltpu.make_async_copy(bwo_hbm.at[h, r], bwo_buf.at[j, s, r],
                                      bwo_sem.at[j]).start(priority=1)

    def lat_store(rows, val):
        for i in range(dc // _LANES):
            lat_buf[i, rows, :] = val[:, i * _LANES:(i + 1) * _LANES]

    def lat_load(rows):
        parts = [lat_buf[i, rows, :] for i in range(dc // _LANES)]
        return jnp.concatenate(parts, axis=1).astype(bf16)

    def widen(w_buf, t):
        rows = w_buf.shape[0] // _WIDEN
        r = _ds(t * rows, rows)
        w32_buf[r, :] = w_buf[r, :].astype(jnp.float32)

    def head_weight(h, n):
        return w32_buf[pl.ds(h, n, stride=nh), :].astype(bf16)

    def query(j):
        xa = _pad_rows(ax_buf[...])
        for h in (2 * j, 2 * j + 1):
            ctx_buf[h] = _dot(xa, head_weight(h, m))

    def absorb(j):
        for h in (2 * j, 2 * j + 1):
            q = ctx_buf[h].astype(bf16)
            lat_store(_ds(h * _ROWS, _ROWS), _dot_nt(q, head_weight(h, dc)))

    nchunk = sk // _KEYS

    def attend(t):
        b, chunk = t // nchunk, t % nchunk
        rows = pl.ds(b, nh, stride=_ROWS)

        @pl.when(chunk == 0)
        def _():
            m_buf[...] = jnp.full(m_buf.shape, -jnp.inf, jnp.float32)
            l_buf[...] = jnp.zeros(l_buf.shape, jnp.float32)
            acc_buf[...] = jnp.zeros(acc_buf.shape, jnp.float32)

        c = ckv_buf[b, _ds(chunk * _KEYS, _KEYS), :]
        s = _dot_nt(lat_load(rows), c) * scale
        m_old = m_buf[...]
        m_new = jnp.maximum(m_old, jnp.max(s, axis=-1, keepdims=True))
        alpha = jnp.exp(m_old - m_new)
        p = jnp.exp(s - m_new[:, :1])
        l_new = alpha * l_buf[...] + jnp.sum(p, axis=-1, keepdims=True)
        acc = alpha[:, :1] * acc_buf[...] + _dot(p.astype(bf16), c)
        m_buf[...] = m_new
        l_buf[...] = l_new
        acc_buf[...] = acc

        @pl.when(chunk == nchunk - 1)
        def _():
            lat_store(rows, acc_buf[...] / l_buf[:, :1])

    def up_project(j):
        for h in (2 * j, 2 * j + 1):
            ctx_buf[h] = _dot(lat_load(_ds(h * _ROWS, _ROWS)), head_weight(h, dc))

    phases = [
        (_WIDEN, lambda t: widen(wq_buf, t)),
        (npair, query),
        (_WIDEN, lambda t: widen(wuk_buf, t)),
        (npair, absorb),
        (nb * nchunk, attend),
        (_WIDEN, lambda t: widen(wuv_buf, t)),
        (npair, up_project),
    ]
    assert sum(n for n, _ in phases) <= nbh

    ax_cp = pltpu.make_async_copy(ax_hbm, ax_buf, io_sem.at[0])
    bx_cp = pltpu.make_async_copy(bx_hbm, bx_buf, io_sem.at[1])
    wbytes = m * nh * dh * 2
    stream_pair(bwq_copy,
                row_copy(wq_hbm, wq_buf, w_sem.at[0], 2 * dh),
                wbytes)
    ax_cp.start()
    bx_cp.start()
    stream_pair(row_copy(wuk_hbm, wuk_buf, w_sem.at[1], 2 * dh),
                row_copy(wuv_hbm, wuv_buf, w_sem.at[2], 2 * dh),
                wbytes)

    bx_cp.wait()
    _wait_all(bwq_buf, w_sem.at[3])
    xb = _pad_rows(bx_buf[...])
    for h in range(nh):
        qb_buf[h] = _dot(xb, bwq_buf[:, h * dh:(h + 1) * dh])
    ob_buf[...] = jnp.zeros(ob_buf.shape, jnp.float32)
    out_acc[...] = jnp.zeros(out_acc.shape, jnp.float32)
    w32_buf[pl.ds(m * nh, nh), :] = jnp.zeros((nh, dh), jnp.float32)
    for i in range(dc // _LANES):
        lat_buf[i, pl.ds(nh * _ROWS, _ROWS), :] = jnp.zeros((_ROWS, _LANES), jnp.float32)

    for b in range(0, nb, 2):
        stream_pair(
            row_copy(ckv_hbm.at[b], ckv_buf.at[b], c_sem.at[b], 2 * dc),
            row_copy(ckv_hbm.at[b + 1], ckv_buf.at[b + 1], c_sem.at[b + 1], 2 * dc),
            sk * dc * 2)

    ahead = _GROUP + _AHEAD

    def first_steps(i, carry):
        kv_issue(i, kv_cuts)
        return carry
    jax.lax.fori_loop(0, ahead, first_steps, 0)

    ax_cp.wait()
    _wait_all(wq_buf, w_sem.at[0])
    _wait_all(wuk_buf, w_sem.at[1])
    _wait_all(wuv_buf, w_sem.at[2])
    for b in range(nb):
        _wait_all(ckv_buf.at[b], c_sem.at[b])

    row = jax.lax.broadcasted_iota(jnp.int32, (_ROWS, dh), 0)
    t_tail = nbh - ahead

    npiece = nstage * stage_pieces
    in_loop = min(_TAIL * ahead, npiece)

    def issue(i, half):
        @pl.when(i < t_tail)
        def _():
            kv_issue(i + ahead, _half(kv_cuts, half))

        for u in _half(range(_TAIL), half):
            piece = (i - t_tail) * _TAIL + u

            @pl.when(jnp.logical_and(i >= t_tail, piece < in_loop))
            def _():
                wo_issue(piece)

    def out_project(j):
        _wait_all(wo_buf.at[j], wo_sem.at[j])
        _wait_all(bwo_buf.at[j], bwo_sem.at[j])
        acc_a, acc_b = out_acc[0], out_acc[1]
        for s in range(_STAGE):
            h = s * nstage + j
            acc_a = acc_a + _dot(ctx_buf[h].astype(bf16), wo_buf[j, s])
            acc_b = acc_b + _dot(ob_buf[h].astype(bf16), bwo_buf[j, s])
        out_acc[0] = acc_a
        out_acc[1] = acc_b

    def head(i, carry):
        g, a = i // _GROUP, i % _GROUP
        slot = g % _SLOTS
        b, h = i // nh, i % nh

        @pl.when(a == 0)
        def _():
            _wait_all(k_buf.at[slot], k_sem.at[slot])
            _wait_all(v_buf.at[slot], v_sem.at[slot])

        s = _dot_nt(qb_buf[h].astype(bf16), k_buf[slot, a]) * scale
        p = jnp.exp(s - jnp.max(s, axis=-1, keepdims=True))
        l = jnp.sum(p, axis=-1, keepdims=True)
        o = _dot(p.astype(bf16), v_buf[slot, a]) / l
        ob_buf[h] = jnp.where(row == b, o, ob_buf[h])

        issue(i, 0)

        first = 0
        for count, piece in phases:
            @pl.when(jnp.logical_and(i >= first, i < first + count))
            def _():
                piece(i - first)
            first += count

        issue(i, 1)

        return carry

    jax.lax.fori_loop(0, nbh, head, 0)
    for piece in range(in_loop, npiece):
        wo_issue(piece, _SPLIT)
    jax.lax.fori_loop(0, nstage, lambda j, c: (out_project(j), c)[1], 0)

    o_buf[:, 0:m] = out_acc[0, 0:nb, :].astype(o_buf.dtype)
    o_buf[:, m:2 * m] = out_acc[1, 0:nb, :].astype(o_buf.dtype)
    o_cp = pltpu.make_async_copy(o_buf, o_hbm, io_sem.at[2])
    o_cp.start()
    o_cp.wait()


@jax.jit
def pallas_concat_heads__compressed_kv_cla__mha_block_cached__decode_kernel(
    A_x: jax.Array,
    A_c_kv: jax.Array,
    A_w_q: jax.Array,
    A_w_uk: jax.Array,
    A_w_uv: jax.Array,
    A_w_o: jax.Array,
    B_x: jax.Array,
    B_k_cache: jax.Array,
    B_v_cache: jax.Array,
    B_wq: jax.Array,
    B_wo: jax.Array,
):
    nb, sq, m = A_x.shape
    _, sk, dc = A_c_kv.shape
    _, nh, dh = A_w_q.shape
    assert sq == 1 and nb <= _ROWS and nb % 2 == 0 and dh == _LANES and dc == m
    assert B_k_cache.shape == (nb, nh, sk, dh) and B_x.shape == A_x.shape
    bf16, f32 = jnp.bfloat16, jnp.float32
    nstage = nh // _STAGE

    hbm = pl.BlockSpec(memory_space=pltpu.HBM)
    out = pl.pallas_call(
        _kernel,
        out_shape=jax.ShapeDtypeStruct((nb, 2 * m), A_x.dtype),
        in_specs=[hbm] * 11,
        out_specs=hbm,
        scratch_shapes=[
            pltpu.VMEM((nb, m), bf16),
            pltpu.VMEM((nb, m), bf16),
            pltpu.VMEM((nb, 2 * m), A_x.dtype),
            pltpu.VMEM((m * nh, dh), bf16),
            pltpu.VMEM((dc * nh, dh), bf16),
            pltpu.VMEM((dc * nh, dh), bf16),
            pltpu.VMEM(((m + 1) * nh, dh), f32),
            pltpu.VMEM((m, nh * dh), bf16),
            pltpu.VMEM((nb, sk, dc), bf16),
            pltpu.VMEM((nstage, _STAGE, dh, m), bf16),
            pltpu.VMEM((nstage, _STAGE, dh, m), bf16),
            pltpu.VMEM((_SLOTS, _GROUP, sk, dh), bf16),
            pltpu.VMEM((_SLOTS, _GROUP, sk, dh), bf16),
            pltpu.VMEM((dc // _LANES, (nh + 1) * _ROWS, _LANES), f32),
            pltpu.VMEM((nh, _LANES), f32),
            pltpu.VMEM((nh, _LANES), f32),
            pltpu.VMEM((nh, dc), f32),
            pltpu.VMEM((nh, _ROWS, dh), f32),
            pltpu.VMEM((nh, _ROWS, dh), f32),
            pltpu.VMEM((nh, _ROWS, dh), f32),
            pltpu.VMEM((2, _ROWS, m), f32),
            pltpu.SemaphoreType.DMA((3,)),
            pltpu.SemaphoreType.DMA((4,)),
            pltpu.SemaphoreType.DMA((nb,)),
            pltpu.SemaphoreType.DMA((nstage,)),
            pltpu.SemaphoreType.DMA((nstage,)),
            pltpu.SemaphoreType.DMA((_SLOTS,)),
            pltpu.SemaphoreType.DMA((_SLOTS,)),
        ],
        compiler_params=pltpu.CompilerParams(
            vmem_limit_bytes=110 * 1024 * 1024,
            disable_bounds_checks=_NOCHECK),
    )(
        A_x.reshape(nb, m), A_c_kv,
        A_w_q.reshape(m * nh, dh),
        A_w_uk.reshape(dc * nh, dh),
        A_w_uv.reshape(dc * nh, dh),
        A_w_o,
        B_x.reshape(nb, m),
        B_k_cache.reshape(nb * nh, sk, dh),
        B_v_cache.reshape(nb * nh, sk, dh),
        B_wq,
        B_wo.reshape(nh, dh, m),
    )
    return out.reshape(nb, sq, 2 * m)
```

```python
import jax
import jax.numpy as jnp
import jax.experimental.pallas as pl
import jax.experimental.pallas.tpu as pltpu

_ROWS = 8
_LANES = 128
_KV_CUTS = (16, 20, 12, 16)
_W_CUTS = (32,)
_WO_KIB = 32
_WAYS = 8
_GROUP = 8
_SLOTS = 3
_AHEAD = 3
_STAGE = 4
_TAIL = 3
_WIDEN = 8
_KEYS = 1024

_NT = (((1,), (1,)), ((), ()))


def _dot(a, b):
    return jnp.dot(a, b, preferred_element_type=jnp.float32)


def _dot_nt(a, b):
    return jax.lax.dot_general(a, b, _NT, preferred_element_type=jnp.float32)


def _pad_rows(x):
    x = x.astype(jnp.float32)
    zeros = jnp.zeros((_ROWS - x.shape[0], x.shape[1]), jnp.float32)
    return jnp.concatenate([x, zeros], axis=0).astype(jnp.bfloat16)


def _ds(start, size):
    if isinstance(start, int):
        return pl.ds(start, size)
    return pl.ds(pl.multiple_of(start, size), size)


def _cut(nbytes, cuts_kib):
    out, off = [], 0
    while off < nbytes:
        size = min(cuts_kib[len(out) % len(cuts_kib)] * 1024, nbytes - off)
        out.append((off, size))
        off += size
    return out


def _half(items, which):
    mid = len(items) // 2
    return items[mid:] if which else items[:mid]


def _wait_all(buf, sem):
    pltpu.make_async_copy(buf, buf, sem).wait()


def _kernel(ax_hbm, ckv_hbm, wq_hbm, wuk_hbm, wuv_hbm, wo_hbm,
            bx_hbm, k_hbm, v_hbm, bwq_hbm, bwo_hbm,
            o_hbm,
            ax_buf, bx_buf, o_buf,
            wq_buf, wuk_buf, wuv_buf, w32_buf, bwq_buf, ckv_buf, wo_buf, bwo_buf,
            k_buf, v_buf,
            lat_buf, m_buf, l_buf, acc_buf, ctx_buf, qb_buf, ob_buf, out_acc,
            io_sem, w_sem, c_sem, wo_sem, bwo_sem, k_sem, v_sem):
    nb, sk, dc = ckv_hbm.shape
    nbh, _, dh = k_hbm.shape
    nh = nbh // nb
    m = ax_hbm.shape[1]
    npair = nh // 2
    scale = dh ** -0.5
    bf16 = jnp.bfloat16

    span = 8 * bwq_hbm.shape[1] * 2

    def row_copy(src, dst, sem, row_bytes):
        per_way = src.shape[0] // _WAYS

        def start(s, c, off, size, queue):
            r0 = s * per_way + c * (span // row_bytes) + off // row_bytes
            r = pl.ds(pl.multiple_of(r0, 8), size // row_bytes)
            pltpu.make_async_copy(src.at[r], dst.at[r], sem).start(priority=queue)
        return start

    def bwq_copy(s, c, off, size, queue):
        r = pl.ds(pl.multiple_of(s * (m // _WAYS) + c * 8, 8), 8)
        cs = pl.ds(off // 16, size // 16)
        pltpu.make_async_copy(bwq_hbm.at[r, cs], bwq_buf.at[r, cs],
                              w_sem.at[3]).start(priority=queue)

    def stream_pair(first, second, nbytes):
        def body(c, carry):
            for off, size in _cut(span, _W_CUTS):
                for s in range(_WAYS):
                    first(s, c, off, size, 0)
                    second(s, c, off, size, 1)
            return carry
        jax.lax.fori_loop(0, nbytes // _WAYS // span, body, 0)

    kv_step = sk // _GROUP
    kv_cuts = _cut(kv_step * 2 * dh, _KV_CUTS)

    def kv_issue(step, cuts):
        g, part = step // _GROUP, step % _GROUP
        slot = g % _SLOTS
        for off, size in cuts:
            r0 = part * kv_step + off // (2 * dh)
            r = pl.ds(pl.multiple_of(r0, 8), size // (2 * dh))
            for a in range(_GROUP):
                pltpu.make_async_copy(k_hbm.at[g * _GROUP + a, r],
                                      k_buf.at[slot, a, r],
                                      k_sem.at[slot]).start(priority=0)
                pltpu.make_async_copy(v_hbm.at[g * _GROUP + a, r],
                                      v_buf.at[slot, a, r],
                                      v_sem.at[slot]).start(priority=1)

    nstage = nh // _STAGE
    wo_rows = _WO_KIB * 1024 // (2 * m)
    stage_pieces = dh // wo_rows

    def wo_issue(piece):
        j = piece // stage_pieces
        r = _ds((piece % stage_pieces) * wo_rows, wo_rows)
        for s in range(_STAGE):
            h = s * nstage + j
            pltpu.make_async_copy(wo_hbm.at[h, r], wo_buf.at[j, s, r],
                                  wo_sem.at[j]).start(priority=0)
            pltpu.make_async_copy(bwo_hbm.at[h, r], bwo_buf.at[j, s, r],
                                  bwo_sem.at[j]).start(priority=1)

    def lat_store(rows, val):
        for i in range(dc // _LANES):
            lat_buf[i, rows, :] = val[:, i * _LANES:(i + 1) * _LANES]

    def lat_load(rows):
        parts = [lat_buf[i, rows, :] for i in range(dc // _LANES)]
        return jnp.concatenate(parts, axis=1).astype(bf16)

    def widen(w_buf, t):
        rows = w_buf.shape[0] // _WIDEN
        r = _ds(t * rows, rows)
        w32_buf[r, :] = w_buf[r, :].astype(jnp.float32)

    def head_weight(h, n):
        return w32_buf[pl.ds(h, n, stride=nh), :].astype(bf16)

    def query(j):
        xa = _pad_rows(ax_buf[...])
        for h in (2 * j, 2 * j + 1):
            ctx_buf[h] = _dot(xa, head_weight(h, m))

    def absorb(j):
        for h in (2 * j, 2 * j + 1):
            q = ctx_buf[h].astype(bf16)
            lat_store(_ds(h * _ROWS, _ROWS), _dot_nt(q, head_weight(h, dc)))

    nchunk = sk // _KEYS

    def attend(t):
        b, chunk = t // nchunk, t % nchunk
        rows = pl.ds(b, nh, stride=_ROWS)

        @pl.when(chunk == 0)
        def _():
            m_buf[...] = jnp.full(m_buf.shape, -jnp.inf, jnp.float32)
            l_buf[...] = jnp.zeros(l_buf.shape, jnp.float32)
            acc_buf[...] = jnp.zeros(acc_buf.shape, jnp.float32)

        c = ckv_buf[b, _ds(chunk * _KEYS, _KEYS), :]
        s = _dot_nt(lat_load(rows), c) * scale
        m_old = m_buf[...]
        m_new = jnp.maximum(m_old, jnp.max(s, axis=-1, keepdims=True))
        alpha = jnp.exp(m_old - m_new)
        p = jnp.exp(s - m_new[:, :1])
        l_new = alpha * l_buf[...] + jnp.sum(p, axis=-1, keepdims=True)
        acc = alpha[:, :1] * acc_buf[...] + _dot(p.astype(bf16), c)
        m_buf[...] = m_new
        l_buf[...] = l_new
        acc_buf[...] = acc

        @pl.when(chunk == nchunk - 1)
        def _():
            lat_store(rows, acc_buf[...] / l_buf[:, :1])

    def up_project(j):
        for h in (2 * j, 2 * j + 1):
            ctx_buf[h] = _dot(lat_load(_ds(h * _ROWS, _ROWS)), head_weight(h, dc))

    phases = [
        (_WIDEN, lambda t: widen(wq_buf, t)),
        (npair, query),
        (_WIDEN, lambda t: widen(wuk_buf, t)),
        (npair, absorb),
        (nb * nchunk, attend),
        (_WIDEN, lambda t: widen(wuv_buf, t)),
        (npair, up_project),
    ]
    assert sum(n for n, _ in phases) <= nbh

    ax_cp = pltpu.make_async_copy(ax_hbm, ax_buf, io_sem.at[0])
    bx_cp = pltpu.make_async_copy(bx_hbm, bx_buf, io_sem.at[1])
    wbytes = m * nh * dh * 2
    stream_pair(bwq_copy,
                row_copy(wq_hbm, wq_buf, w_sem.at[0], 2 * dh),
                wbytes)
    ax_cp.start()
    bx_cp.start()
    stream_pair(row_copy(wuk_hbm, wuk_buf, w_sem.at[1], 2 * dh),
                row_copy(wuv_hbm, wuv_buf, w_sem.at[2], 2 * dh),
                wbytes)

    bx_cp.wait()
    _wait_all(bwq_buf, w_sem.at[3])
    xb = _pad_rows(bx_buf[...])
    for h in range(nh):
        qb_buf[h] = _dot(xb, bwq_buf[:, h * dh:(h + 1) * dh])
    ob_buf[...] = jnp.zeros(ob_buf.shape, jnp.float32)
    out_acc[...] = jnp.zeros(out_acc.shape, jnp.float32)
    w32_buf[pl.ds(m * nh, nh), :] = jnp.zeros((nh, dh), jnp.float32)
    for i in range(dc // _LANES):
        lat_buf[i, pl.ds(nh * _ROWS, _ROWS), :] = jnp.zeros(
            (_ROWS, _LANES), jnp.float32)

    for b in range(0, nb, 2):
        stream_pair(
            row_copy(ckv_hbm.at[b], ckv_buf.at[b], c_sem.at[b], 2 * dc),
            row_copy(ckv_hbm.at[b + 1], ckv_buf.at[b + 1], c_sem.at[b + 1], 2 * dc),
            sk * dc * 2)

    ahead = _GROUP + _AHEAD
    assert ahead <= (_SLOTS - 1) * _GROUP

    def first_steps(i, carry):
        kv_issue(i, kv_cuts)
        return carry
    jax.lax.fori_loop(0, ahead, first_steps, 0)

    ax_cp.wait()
    _wait_all(wq_buf, w_sem.at[0])
    _wait_all(wuk_buf, w_sem.at[1])
    _wait_all(wuv_buf, w_sem.at[2])
    for b in range(nb):
        _wait_all(ckv_buf.at[b], c_sem.at[b])

    row = jax.lax.broadcasted_iota(jnp.int32, (_ROWS, dh), 0)
    t_tail = nbh - ahead
    npiece = nstage * stage_pieces
    in_loop = min(_TAIL * ahead, npiece)

    def issue(i, half):
        @pl.when(i < t_tail)
        def _():
            kv_issue(i + ahead, _half(kv_cuts, half))

        for u in _half(range(_TAIL), half):
            piece = (i - t_tail) * _TAIL + u

            @pl.when(jnp.logical_and(i >= t_tail, piece < in_loop))
            def _():
                wo_issue(piece)

    def out_project(j):
        _wait_all(wo_buf.at[j], wo_sem.at[j])
        _wait_all(bwo_buf.at[j], bwo_sem.at[j])
        acc_a, acc_b = out_acc[0], out_acc[1]
        for s in range(_STAGE):
            h = s * nstage + j
            acc_a = acc_a + _dot(ctx_buf[h].astype(bf16), wo_buf[j, s])
            acc_b = acc_b + _dot(ob_buf[h].astype(bf16), bwo_buf[j, s])
        out_acc[0] = acc_a
        out_acc[1] = acc_b

    def head(i, carry):
        g, a = i // _GROUP, i % _GROUP
        slot = g % _SLOTS
        b, h = i // nh, i % nh

        @pl.when(a == 0)
        def _():
            _wait_all(k_buf.at[slot], k_sem.at[slot])
            _wait_all(v_buf.at[slot], v_sem.at[slot])

        s = _dot_nt(qb_buf[h].astype(bf16), k_buf[slot, a]) * scale
        p = jnp.exp(s - jnp.max(s, axis=-1, keepdims=True))
        l = jnp.sum(p, axis=-1, keepdims=True)
        o = _dot(p.astype(bf16), v_buf[slot, a]) / l
        ob_buf[h] = jnp.where(row == b, o, ob_buf[h])

        issue(i, 0)

        first = 0
        for count, piece in phases:
            @pl.when(jnp.logical_and(i >= first, i < first + count))
            def _():
                piece(i - first)
            first += count

        issue(i, 1)

        return carry

    jax.lax.fori_loop(0, nbh, head, 0)
    for piece in range(in_loop, npiece):
        wo_issue(piece)
    jax.lax.fori_loop(0, nstage, lambda j, c: (out_project(j), c)[1], 0)

    o_buf[:, 0:m] = out_acc[0, 0:nb, :].astype(o_buf.dtype)
    o_buf[:, m:2 * m] = out_acc[1, 0:nb, :].astype(o_buf.dtype)
    o_cp = pltpu.make_async_copy(o_buf, o_hbm, io_sem.at[2])
    o_cp.start()
    o_cp.wait()


@jax.jit
def pallas_concat_heads__compressed_kv_cla__mha_block_cached__decode_kernel(
    A_x: jax.Array,
    A_c_kv: jax.Array,
    A_w_q: jax.Array,
    A_w_uk: jax.Array,
    A_w_uv: jax.Array,
    A_w_o: jax.Array,
    B_x: jax.Array,
    B_k_cache: jax.Array,
    B_v_cache: jax.Array,
    B_wq: jax.Array,
    B_wo: jax.Array,
):
    nb, sq, m = A_x.shape
    _, sk, dc = A_c_kv.shape
    _, nh, dh = A_w_q.shape
    assert sq == 1 and nb <= _ROWS and nb % 2 == 0 and dh == _LANES and dc == m
    assert B_k_cache.shape == (nb, nh, sk, dh) and B_x.shape == A_x.shape
    assert m % (8 * _WAYS) == 0 and (sk * dc) % (8 * _WAYS * nh * dh) == 0
    assert nh % _GROUP == 0 and nh % _STAGE == 0 and (m * nh) % (16 * _WIDEN) == 0
    assert sk % (16 * _GROUP) == 0 and sk % _KEYS == 0
    assert (dh * 2 * m) % (_WO_KIB * 1024) == 0 and (_WO_KIB * 1024) % (32 * m) == 0
    bf16, f32 = jnp.bfloat16, jnp.float32
    nstage = nh // _STAGE

    hbm = pl.BlockSpec(memory_space=pltpu.HBM)
    out = pl.pallas_call(
        _kernel,
        out_shape=jax.ShapeDtypeStruct((nb, 2 * m), A_x.dtype),
        in_specs=[hbm] * 11,
        out_specs=hbm,
        scratch_shapes=[
            pltpu.VMEM((nb, m), bf16),
            pltpu.VMEM((nb, m), bf16),
            pltpu.VMEM((nb, 2 * m), A_x.dtype),
            pltpu.VMEM((m * nh, dh), bf16),
            pltpu.VMEM((dc * nh, dh), bf16),
            pltpu.VMEM((dc * nh, dh), bf16),
            pltpu.VMEM(((m + 1) * nh, dh), f32),
            pltpu.VMEM((m, nh * dh), bf16),
            pltpu.VMEM((nb, sk, dc), bf16),
            pltpu.VMEM((nstage, _STAGE, dh, m), bf16),
            pltpu.VMEM((nstage, _STAGE, dh, m), bf16),
            pltpu.VMEM((_SLOTS, _GROUP, sk, dh), bf16),
            pltpu.VMEM((_SLOTS, _GROUP, sk, dh), bf16),
            pltpu.VMEM((dc // _LANES, (nh + 1) * _ROWS, _LANES), f32),
            pltpu.VMEM((nh, _LANES), f32),
            pltpu.VMEM((nh, _LANES), f32),
            pltpu.VMEM((nh, dc), f32),
            pltpu.VMEM((nh, _ROWS, dh), f32),
            pltpu.VMEM((nh, _ROWS, dh), f32),
            pltpu.VMEM((nh, _ROWS, dh), f32),
            pltpu.VMEM((2, _ROWS, m), f32),
            pltpu.SemaphoreType.DMA((3,)),
            pltpu.SemaphoreType.DMA((4,)),
            pltpu.SemaphoreType.DMA((nb,)),
            pltpu.SemaphoreType.DMA((nstage,)),
            pltpu.SemaphoreType.DMA((nstage,)),
            pltpu.SemaphoreType.DMA((_SLOTS,)),
            pltpu.SemaphoreType.DMA((_SLOTS,)),
        ],
        compiler_params=pltpu.CompilerParams(
            vmem_limit_bytes=110 * 1024 * 1024,
            disable_bounds_checks=True),
    )(
        A_x.reshape(nb, m), A_c_kv,
        A_w_q.reshape(m * nh, dh),
        A_w_uk.reshape(dc * nh, dh),
        A_w_uv.reshape(dc * nh, dh),
        A_w_o,
        B_x.reshape(nb, m),
        B_k_cache.reshape(nb * nh, sk, dh),
        B_v_cache.reshape(nb * nh, sk, dh),
        B_wq,
        B_wo.reshape(nh, dh, m),
    )
    return out.reshape(nb, sq, 2 * m)
```
